```python
import os as _os
_os.environ.setdefault('JAX_PLATFORMS', 'cpu')
import jax
import jax.numpy as jnp

def _softmax(x, axis=-1):
    return jax.nn.softmax(x, axis=axis)

def _gelu(x):
    return jax.nn.gelu(x, approximate=True)

def _silu(x):
    return jax.nn.silu(x)

def _sigmoid(x):
    return jax.nn.sigmoid(x)

def _layernorm(x, axis=-1, eps=1e-05):
    m = jnp.mean(x, axis=axis, keepdims=True)
    v = jnp.var(x, axis=axis, keepdims=True)
    return (x - m) / jnp.sqrt(v + eps)

def _scatter_add(tgt, idx, src, axis=0):
    return tgt.at[idx].add(src)

def _segment_sum(src, seg, n):
    return jax.ops.segment_sum(src, seg, n)

class _Rng:

    def __init__(self, key):
        self._k = key

    def _next(self):
        self._k, sub = jax.random.split(self._k)
        return sub

    def normal(self, shape):
        return jax.random.normal(self._next(), shape, dtype=jnp.bfloat16)

    def randint(self, lo, hi, shape):
        return jax.random.randint(self._next(), shape, lo, hi, dtype=jnp.int32)

    def uniform(self, shape, lo=0.0, hi=1.0):
        return jax.random.uniform(self._next(), shape, jnp.bfloat16, lo, hi)

    def permutation(self, n):
        return jax.random.permutation(self._next(), n)
kernel_name = 'sequential_preLN__linear_attn_block__mixer_gmlp__prompt'

def setup_inputs():
    _rng = _Rng(jax.random.key(int.from_bytes(__import__("os").urandom(4), "little")))
    _w = lambda a: (lambda t: t.astype(jnp.bfloat16) if jnp.issubdtype(t.dtype, jnp.floating) else t)(jnp.asarray(a))

    def _A_setup():
        B, S, D = (1, 2048, 512)
        return {'x': _w((lambda *s: _rng.normal(s) * 0.05)(B, S, D)), 'wqkv': _w((lambda *s: _rng.normal(s) * 0.05)(D, 3 * D)), 'wo': _w((lambda *s: _rng.normal(s) * 0.05)(D, D))}
    _A_in = _A_setup()

    def _B_setup():
        B, S, D, F = (1, 2048, 512, 1792)
        Fh = F // 2
        return {'x': _w((lambda *s: _rng.normal(s) * 0.05)(B, S, D)), 'w_in': _w((lambda *s: _rng.normal(s) * 0.4)(D, 2 * Fh)), 'w_sp': _w(0.01 * (lambda *s: _rng.normal(s) * 0.4)(S, S)), 'b_sp': _w(1.0 + 0.01 * (lambda *s: _rng.normal(s) * 0.05)(S)), 'w_out': _w((lambda *s: _rng.normal(s) * 0.05)(Fh, D))}
    _B_in = _B_setup()
    return {'A_x': _A_in['x'], 'A_wqkv': _A_in['wqkv'], 'A_wo': _A_in['wo'], 'B_x': _B_in['x'], 'B_w_in': _B_in['w_in'], 'B_w_sp': _B_in['w_sp'], 'B_b_sp': _B_in['b_sp'], 'B_w_out': _B_in['w_out']}

def reference(A_x, A_wqkv, A_wo, B_x, B_w_in, B_w_sp, B_b_sp, B_w_out):

    def _A_ref(x, wqkv, wo):
        B, S, D = x.shape
        H = 32
        Dh = D // H
        qkv = (lambda x, *d: x.transpose(*d))((x @ wqkv).reshape(B, S, 3, H, Dh), 2, 0, 3, 1, 4)
        q, k, v = (qkv[0], qkv[1], qkv[2])
        phi = lambda t: jnp.where(t > 0, t + 1, jnp.exp(t)) + 1e-06
        pq, pk = (phi(q), phi(k))
        kv = jnp.einsum('bhsd,bhse->bhde', pk, v)
        z = jnp.einsum('bhsd->bhd', pk)
        num = jnp.einsum('bhqd,bhde->bhqe', pq, kv)
        den = jnp.einsum('bhqd,bhd->bhq', pq, z)[..., None] + 1e-06
        o = num / den
        return (lambda x, *d: x.transpose(*d))(o, 0, 2, 1, 3).reshape(B, S, D) @ wo

    def _B_ref(x, w_in, w_sp, b_sp, w_out):
        B, S, D = x.shape
        F = w_in.shape[-1]
        Fh = F // 2
        z = _gelu(jnp.einsum('bsd,df->bsf', x, w_in))
        z1 = z[..., :Fh].copy()
        z2 = _layernorm(z[..., Fh:], axis=-1)
        g = jnp.einsum('ts,bsf->btf', w_sp, z2) + b_sp[None, :, None]
        return jnp.einsum('bsf,fd->bsd', z1 * g, w_out)
    x = A_x
    h = x + _A_ref(_layernorm(x, axis=-1), A_wqkv, A_wo)
    h2 = h + _B_ref(_layernorm(h, axis=-1), B_w_in, B_w_sp, B_b_sp, B_w_out)
    return h2
```

```python
import functools

import jax
import jax.numpy as jnp
from jax import lax
import jax.experimental.pallas as pl
import jax.experimental.pallas.tpu as pltpu

_BF16 = jnp.bfloat16
_F32 = jnp.float32

_LANES = 128
_HEAD_DIM = 16
_TM = 256


def _ln(x):
    mu = jnp.mean(x, axis=-1, keepdims=True)
    xc = x - mu
    var = jnp.mean(xc * xc, axis=-1, keepdims=True)
    return xc * lax.rsqrt(var + 1e-5)


def _phi(t):
    return jnp.where(t > 0, t + 1.0, jnp.exp(t)) + 1e-6


def _gelu(x):
    c = 0.7978845608028654
    return 0.5 * x * (1.0 + jnp.tanh(c * (x + 0.044715 * (x * x * x))))


def _dot(a, b):
    return jnp.dot(a, b, preferred_element_type=_F32)


def _kernel(x_hbm, wqkv_hbm, wo_hbm, win_hbm, wsp_hbm, bsp_hbm, wout_hbm,
            out_hbm,
            x_v, wqkv_v, wo_v, win_v, wsp_v, bsp_v, wout_v,
            pq_v, h_v, z1_v, z2_v, o_v, kv_v, zs_v, m_v, zm_v,
            sem_x, sem_w, sem_sp, sem_o):
    S, D = x_v.shape
    FH = z1_v.shape[1]
    TM = _TM
    NT = S // TM
    NB = D // _LANES

    def x_copy(i):
        return pltpu.make_async_copy(
            x_hbm.at[pl.ds(i * TM, TM)], x_v.at[pl.ds(i * TM, TM)], sem_x.at[i])

    def sp_copy(i):
        return pltpu.make_async_copy(
            wsp_hbm.at[pl.ds(i * TM, TM)], wsp_v.at[pl.ds(i * TM, TM)], sem_sp.at[i])

    def o_copy(i):
        return pltpu.make_async_copy(
            o_v.at[pl.ds(i * TM, TM)], out_hbm.at[pl.ds(i * TM, TM)], sem_o.at[i])

    c_wqkv = pltpu.make_async_copy(wqkv_hbm, wqkv_v, sem_w.at[0])
    c_wo = pltpu.make_async_copy(wo_hbm, wo_v, sem_w.at[1])
    c_win = pltpu.make_async_copy(win_hbm, win_v, sem_w.at[2])
    c_wout = pltpu.make_async_copy(wout_hbm, wout_v, sem_w.at[3])
    c_bsp = pltpu.make_async_copy(bsp_hbm, bsp_v, sem_w.at[4])

    x_copy(0).start()
    c_wqkv.start()
    for i in range(1, NT):
        x_copy(i).start()
    c_wo.start()
    c_win.start()
    c_bsp.start()
    c_wout.start()
    for i in range(NT):
        sp_copy(i).start()

    kv_v[...] = jnp.zeros(kv_v.shape, _F32)
    zs_v[...] = jnp.zeros(zs_v.shape, _F32)
    c_wqkv.wait()

    def phase1(i, carry):
        r0 = pl.multiple_of(i * TM, TM)
        rows = pl.ds(r0, TM)
        x_copy(i).wait()
        xn = _ln(x_v[rows, :].astype(_F32)).astype(_BF16)
        qkv = _dot(xn, wqkv_v[...])
        pq_v[rows, :] = _phi(qkv[:, :D]).astype(_BF16)
        pk = _phi(qkv[:, D:2 * D])
        zs_v[...] += jnp.sum(pk, axis=0, keepdims=True)
        pkb = pk.astype(_BF16)
        vb = qkv[:, 2 * D:].astype(_BF16)
        for b in range(NB):
            cols = slice(b * _LANES, (b + 1) * _LANES)
            kv_v[b] += lax.dot_general(
                pkb[:, cols], vb[:, cols], (((0,), (0,)), ((), ())),
                preferred_element_type=_F32)
        return carry

    lax.fori_loop(0, NT, phase1, 0)

    c_wo.wait()
    ri = lax.broadcasted_iota(jnp.int32, (_LANES, _LANES), 0) // _HEAD_DIM
    ci = lax.broadcasted_iota(jnp.int32, (_LANES, _LANES), 1) // _HEAD_DIM
    same_head = ri == ci
    for b in range(NB):
        cols = slice(b * _LANES, (b + 1) * _LANES)
        kvm = jnp.where(same_head, kv_v[b], 0.0).astype(_BF16)
        m_v[cols, :] = _dot(kvm, wo_v[cols, :]).astype(_BF16)
        zrow = jnp.broadcast_to(zs_v[:, cols], (_LANES, _LANES))
        zm_v[b] = jnp.where(same_head, zrow.T, 0.0).astype(_BF16)

    c_win.wait()

    def phase2(i, carry):
        r0 = pl.multiple_of(i * TM, TM)
        rows = pl.ds(r0, TM)
        pq = pq_v[rows, :]
        den = jnp.concatenate(
            [_dot(pq[:, b * _LANES:(b + 1) * _LANES], zm_v[b]) for b in range(NB)],
            axis=1) + 1e-6
        pqs = (pq.astype(_F32) / den).astype(_BF16)
        h = x_v[rows, :].astype(_F32) + _dot(pqs, m_v[...])
        h_v[rows, :] = h
        hn = _ln(h).astype(_BF16)
        z1_v[rows, :] = _gelu(_dot(hn, win_v[:, :FH])).astype(_BF16)
        z2_v[rows, :] = _ln(_gelu(_dot(hn, win_v[:, FH:]))).astype(_BF16)
        return carry

    lax.fori_loop(0, NT, phase2, 0)

    c_wout.wait()
    c_bsp.wait()

    def phase3(i, carry):
        r0 = pl.multiple_of(i * TM, TM)
        rows = pl.ds(r0, TM)
        sp_copy(i).wait()
        brow = bsp_v[:, rows].astype(_F32)
        bcol = jnp.broadcast_to(brow, (_LANES, TM)).T
        bfull = jnp.concatenate([bcol] * (FH // _LANES), axis=1)
        g = _dot(wsp_v[rows, :], z2_v[...]) + bfull
        u = (z1_v[rows, :].astype(_F32) * g).astype(_BF16)
        o_v[rows, :] = (h_v[rows, :] + _dot(u, wout_v[...])).astype(_BF16)
        o_copy(i).start()
        return carry

    lax.fori_loop(0, NT, phase3, 0)
    for i in range(NT):
        o_copy(i).wait()


@jax.jit
def pallas_sequential_preLN__linear_attn_block__mixer_gmlp__prompt_kernel(
    A_x: jax.Array,
    A_wqkv: jax.Array,
    A_wo: jax.Array,
    B_x: jax.Array,
    B_w_in: jax.Array,
    B_w_sp: jax.Array,
    B_b_sp: jax.Array,
    B_w_out: jax.Array,
):
    B, S, D = A_x.shape
    FH = B_w_out.shape[0]
    NT = S // _TM
    NB = D // _LANES
    x2 = A_x.reshape(S, D)
    bsp2 = B_b_sp.reshape(1, S)
    any_spec = pl.BlockSpec(memory_space=pl.ANY)
    out = pl.pallas_call(
        _kernel,
        out_shape=jax.ShapeDtypeStruct((S, D), _BF16),
        in_specs=[any_spec] * 7,
        out_specs=any_spec,
        scratch_shapes=[
            pltpu.VMEM((S, D), _BF16),
            pltpu.VMEM((D, 3 * D), _BF16),
            pltpu.VMEM((D, D), _BF16),
            pltpu.VMEM((D, 2 * FH), _BF16),
            pltpu.VMEM((S, S), _BF16),
            pltpu.VMEM((1, S), _BF16),
            pltpu.VMEM((FH, D), _BF16),
            pltpu.VMEM((S, D), _BF16),
            pltpu.VMEM((S, D), _F32),
            pltpu.VMEM((S, FH), _BF16),
            pltpu.VMEM((S, FH), _BF16),
            pltpu.VMEM((S, D), _BF16),
            pltpu.VMEM((NB, _LANES, _LANES), _F32),
            pltpu.VMEM((1, D), _F32),
            pltpu.VMEM((D, D), _BF16),
            pltpu.VMEM((NB, _LANES, _LANES), _BF16),
            pltpu.SemaphoreType.DMA((NT,)),
            pltpu.SemaphoreType.DMA((5,)),
            pltpu.SemaphoreType.DMA((NT,)),
            pltpu.SemaphoreType.DMA((NT,)),
        ],
        compiler_params=pltpu.CompilerParams(vmem_limit_bytes=100 * 1024 * 1024),
    )(x2, A_wqkv, A_wo, B_w_in, B_w_sp, bsp2, B_w_out)
    return out.reshape(B, S, D)
```

```python
import jax
import jax.numpy as jnp
from jax import lax
import jax.experimental.pallas as pl
import jax.experimental.pallas.tpu as pltpu

_BF16 = jnp.bfloat16
_F32 = jnp.float32

_LANES = 128
_HEAD_DIM = 16
_TM = 256
_NDEF = 2
_QSPLIT = 2
_SLOTS = (2, 0, 0, 2, 4)


def _ln(x):
    inv_n = 1.0 / x.shape[-1]
    mu = jnp.sum(x, axis=-1, keepdims=True) * inv_n
    xc = x - mu
    var = jnp.sum(xc * xc, axis=-1, keepdims=True) * inv_n
    return xc * lax.rsqrt(var + 1e-5)


def _phi(t):
    return jnp.where(t > 0, t + 1.0, jnp.exp(t)) + 1e-6


def _gelu(x):
    c = 0.7978845608028654
    inner = x * (c + (c * 0.044715) * (x * x))
    hx = 0.5 * x
    return hx + hx * jnp.tanh(inner)


def _head_sum(t):
    w = t
    s = 1
    while s < _HEAD_DIM:
        w = w + pltpu.roll(w, s, 1)
        s *= 2
    lane = lax.broadcasted_iota(jnp.int32, t.shape, 1)
    m = jnp.where(lane % _HEAD_DIM == _HEAD_DIM - 1, w, 0.0)
    s = 1
    while s < _HEAD_DIM:
        m = m + pltpu.roll(m, _LANES - s, 1)
        s *= 2
    return m


def _recip(d):
    r = pl.reciprocal(d, approx=True)
    return r * (2.0 - d * r)


def _dot(a, b):
    return jnp.dot(a, b, preferred_element_type=_F32)


def _kernel(x_hbm, wqkv_hbm, wo_hbm, win_hbm, wsp_hbm, bsp_hbm, wout_hbm,
            out_hbm,
            x_v, wqkv_v, wo_v, win_v, wsp_v, bsp_v, wout_v,
            pq_v, pqs_v, h_v, z1_v, z2_v, g_v, o_v, kv_v, zs_v, m_v, zm_v,
            sem_in, sem_o):
    S, D = x_v.shape
    FH = z1_v.shape[1]
    TM = _TM
    NT = S // TM
    NB = D // _LANES
    GR = S // sum(_SLOTS)
    QW = D // _QSPLIT
    HT = TM // 2

    def tile(i):
        if isinstance(i, int):
            return pl.ds(i * TM, TM)
        return pl.ds(pl.multiple_of(i * TM, TM), TM)

    def rows_copy(src, dst, r0, n, sem):
        return pltpu.make_async_copy(src.at[pl.ds(r0, n)], dst.at[pl.ds(r0, n)], sem)

    def cols_copy(src, dst, c0, n, sem):
        return pltpu.make_async_copy(src.at[:, pl.ds(c0, n)], dst.at[:, pl.ds(c0, n)], sem)

    c_x0 = rows_copy(x_hbm, x_v, 0, TM, sem_in.at[0])
    c_x1 = rows_copy(x_hbm, x_v, TM, TM, sem_in.at[1])
    c_x24 = rows_copy(x_hbm, x_v, 2 * TM, 3 * TM, sem_in.at[2])
    c_xr = rows_copy(x_hbm, x_v, 5 * TM, S - 5 * TM, sem_in.at[11])
    c_wk = cols_copy(wqkv_hbm, wqkv_v, D, D, sem_in.at[3])
    c_wv = cols_copy(wqkv_hbm, wqkv_v, 2 * D, D, sem_in.at[4])
    c_wq = cols_copy(wqkv_hbm, wqkv_v, 0, D, sem_in.at[5])
    c_wo = pltpu.make_async_copy(wo_hbm, wo_v, sem_in.at[6])
    c_win = pltpu.make_async_copy(win_hbm, win_v, sem_in.at[7])
    c_wout = pltpu.make_async_copy(wout_hbm, wout_v, sem_in.at[8])
    c_bsp = pltpu.make_async_copy(bsp_hbm, bsp_v, sem_in.at[9])
    c_wsp = pltpu.make_async_copy(wsp_hbm, wsp_v, sem_in.at[10])
    o_copies = [rows_copy(o_v, out_hbm, i * TM, TM, sem_o.at[i]) for i in range(NT - 1)]
    o_copies += [rows_copy(o_v, out_hbm, (NT - 1) * TM + j * HT, HT, sem_o.at[NT - 1 + j])
                 for j in range(2)]

    for c in (c_x0, c_wk, c_wv, c_x1, c_wq, c_x24):
        c.start()
    kv_v[...] = jnp.zeros(kv_v.shape, _F32)
    zs_v[...] = jnp.zeros(zs_v.shape, _F32)
    c_x0.wait()
    xn = _ln(x_v[tile(0), :].astype(_F32)).astype(_BF16)
    c_wk.wait()

    deferred = []

    def qpiece():
        if deferred:
            i, c, xn_i = deferred.pop(0)
            qc = _dot(xn_i, wqkv_v[:, c * QW:(c + 1) * QW])
            pq_v[tile(i), c * QW:(c + 1) * QW] = _phi(qc).astype(_BF16)

    for i in range(NT):
        k = _dot(xn, wqkv_v[:, D:2 * D])
        if i == 0:
            c_wv.wait()
        v = _dot(xn, wqkv_v[:, 2 * D:])
        if i == 0:
            c_x1.wait()
            c_wq.wait()
            for c in (c_xr, c_wo, c_win, c_bsp, c_wout, c_wsp):
                c.start()
        g_v[tile(i), :] = jnp.zeros((TM, FH), _F32)
        pk = _phi(k)
        pkb = pk.astype(_BF16)
        vb = v.astype(_BF16)
        defer = i >= NT - _NDEF
        if defer:
            for c in range(_QSPLIT):
                deferred.append((i, c, xn))
        else:
            q = _dot(xn, wqkv_v[:, :D])
        if i + 1 < NT:
            xn = _ln(x_v[tile(i + 1), :].astype(_F32)).astype(_BF16)
        zs_v[...] += jnp.sum(pk, axis=0, keepdims=True)
        for b in range(NB):
            cols = slice(b * _LANES, (b + 1) * _LANES)
            kv_v[b] += lax.dot_general(
                pkb[:, cols], vb[:, cols], (((0,), (0,)), ((), ())),
                preferred_element_type=_F32)
        if not defer:
            pq_v[tile(i), :] = _phi(q).astype(_BF16)
        if i == 0:
            c_x24.wait()
        if i == 3:
            for c in (c_xr, c_wo, c_win, c_bsp, c_wout):
                c.wait()

    qpiece()
    ri = lax.broadcasted_iota(jnp.int32, (_LANES, _LANES), 0) // _HEAD_DIM
    ci = lax.broadcasted_iota(jnp.int32, (_LANES, _LANES), 1) // _HEAD_DIM
    same_head = ri == ci
    for b in range(NB):
        cols = slice(b * _LANES, (b + 1) * _LANES)
        zrow = jnp.broadcast_to(zs_v[:, cols], (_LANES, _LANES))
        zm_v[b] = jnp.where(same_head, zrow.T, 0.0).astype(_BF16)
    for b in range(NB):
        cols = slice(b * _LANES, (b + 1) * _LANES)
        kvm = jnp.where(same_head, kv_v[b], 0.0).astype(_BF16)
        m_v[cols, :] = _dot(kvm, wo_v[cols, :]).astype(_BF16)

    def norm_q(i):
        pqf = pq_v[tile(i), :].astype(_F32)
        t = pqf * zs_v[...]
        den = jnp.concatenate(
            [_head_sum(t[:, b * _LANES:(b + 1) * _LANES]) for b in range(NB)],
            axis=1) + 1e-6
        pqs_v[tile(i), :] = (pqf * _recip(den)).astype(_BF16)

    def phase2(i, with_g):
        rows = tile(i)
        if with_g:
            prev = tile(i - 1)
            zprev = z2_v[prev, :]
        count = [0]

        def gslot(n):
            if with_g:
                for _ in range(n):
                    r = slice(count[0] * GR, (count[0] + 1) * GR)
                    count[0] += 1
                    g_v[r, :] += _dot(wsp_v[r, prev], zprev)
            elif n:
                qpiece()

        nxt = min(i + 1, NT - 1) if isinstance(i, int) else jnp.minimum(i + 1, NT - 1)
        if with_g:
            pqs = pqs_v[rows, :]
        else:
            pq = pq_v[rows, :]
            den = jnp.concatenate(
                [_dot(pq[:, b * _LANES:(b + 1) * _LANES], zm_v[b]) for b in range(NB)],
                axis=1) + 1e-6
            qpiece()
            pqs = (pq.astype(_F32) * _recip(den)).astype(_BF16)
        h = x_v[rows, :].astype(_F32) + _dot(pqs, m_v[...])
        gslot(_SLOTS[0])
        h_v[rows, :] = h
        hn = _ln(h).astype(_BF16)
        norm_q(nxt)
        gslot(_SLOTS[1])
        a1 = _dot(hn, win_v[:, :FH])
        z1_v[rows, :] = _gelu(a1).astype(_BF16)
        gslot(_SLOTS[2])
        a2 = _dot(hn, win_v[:, FH:])
        gslot(_SLOTS[3])
        z2_v[rows, :] = _ln(_gelu(a2)).astype(_BF16)
        gslot(_SLOTS[4])

    phase2(0, False)
    while deferred:
        qpiece()
    c_wsp.wait()

    def phase2_loop(i, carry):
        phase2(i, True)
        return carry

    lax.fori_loop(1, NT, phase2_loop, 0)

    last = tile(NT - 1)
    zlast = z2_v[last, :]
    RB = TM // _LANES

    def gate(i):
        rows = tile(i)
        bcol = jnp.concatenate(
            [jnp.broadcast_to(bsp_v[i * RB + j:i * RB + j + 1, :].astype(_F32),
                              (_LANES, _LANES)).T for j in range(RB)], axis=0)
        bfull = jnp.concatenate([bcol] * (FH // _LANES), axis=1)
        return g_v[rows, :] + bfull + _dot(wsp_v[rows, last], zlast)

    def gated(i, g):
        return (z1_v[tile(i), :].astype(_F32) * g).astype(_BF16)

    u = gated(0, gate(0))
    for i in range(NT - 1):
        gn = gate(i + 1)
        o = h_v[tile(i), :] + _dot(u, wout_v[...])
        u = gated(i + 1, gn)
        o_v[tile(i), :] = o.astype(_BF16)
        o_copies[i].start()
    for j in range(2):
        r = pl.ds((NT - 1) * TM + j * HT, HT)
        o = h_v[r, :] + _dot(u[j * HT:(j + 1) * HT], wout_v[...])
        o_v[r, :] = o.astype(_BF16)
        o_copies[NT - 1 + j].start()
    for c in o_copies:
        c.wait()


@jax.jit
def pallas_sequential_preLN__linear_attn_block__mixer_gmlp__prompt_kernel(
    A_x: jax.Array,
    A_wqkv: jax.Array,
    A_wo: jax.Array,
    B_x: jax.Array,
    B_w_in: jax.Array,
    B_w_sp: jax.Array,
    B_b_sp: jax.Array,
    B_w_out: jax.Array,
):
    del B_x
    B, S, D = A_x.shape
    FH = B_w_out.shape[0]
    NT = S // _TM
    NB = D // _LANES
    x2 = A_x.reshape(S, D)
    bsp2 = B_b_sp.reshape(S // _LANES, _LANES)
    any_spec = pl.BlockSpec(memory_space=pl.ANY)
    out = pl.pallas_call(
        _kernel,
        out_shape=jax.ShapeDtypeStruct((S, D), _BF16),
        in_specs=[any_spec] * 7,
        out_specs=any_spec,
        scratch_shapes=[
            pltpu.VMEM((S, D), _BF16),
            pltpu.VMEM((D, 3 * D), _BF16),
            pltpu.VMEM((D, D), _BF16),
            pltpu.VMEM((D, 2 * FH), _BF16),
            pltpu.VMEM((S, S), _BF16),
            pltpu.VMEM((S // _LANES, _LANES), _BF16),
            pltpu.VMEM((FH, D), _BF16),
            pltpu.VMEM((S, D), _BF16),
            pltpu.VMEM((S, D), _BF16),
            pltpu.VMEM((S, D), _F32),
            pltpu.VMEM((S, FH), _BF16),
            pltpu.VMEM((S, FH), _BF16),
            pltpu.VMEM((S, FH), _F32),
            pltpu.VMEM((S, D), _BF16),
            pltpu.VMEM((NB, _LANES, _LANES), _F32),
            pltpu.VMEM((1, D), _F32),
            pltpu.VMEM((D, D), _BF16),
            pltpu.VMEM((NB, _LANES, _LANES), _BF16),
            pltpu.SemaphoreType.DMA((12,)),
            pltpu.SemaphoreType.DMA((NT + 1,)),
        ],
        compiler_params=pltpu.CompilerParams(vmem_limit_bytes=100 * 1024 * 1024),
    )(x2, A_wqkv, A_wo, B_w_in, B_w_sp, bsp2, B_w_out)
    return out.reshape(B, S, D)
```
